```python
import os as _os
_os.environ.setdefault("JAX_PLATFORMS", "cpu")
import jax
import jax.numpy as jnp

def _softmax(x, axis=-1):
    return jax.nn.softmax(x, axis=axis)
def _gelu(x):
    return jax.nn.gelu(x, approximate=True)
def _silu(x):
    return jax.nn.silu(x)
def _sigmoid(x):
    return jax.nn.sigmoid(x)
def _layernorm(x, axis=-1, eps=1e-5):
    m = jnp.mean(x, axis=axis, keepdims=True)
    v = jnp.var(x, axis=axis, keepdims=True)
    return (x - m) / jnp.sqrt(v + eps)
def _scatter_add(tgt, idx, src, axis=0):
    return tgt.at[idx].add(src)
def _segment_sum(src, seg, n):
    return jax.ops.segment_sum(src, seg, n)
class _Rng:
    def __init__(self, key):
        self._k = key
    def _next(self):
        self._k, sub = jax.random.split(self._k)
        return sub
    def normal(self, shape):
        return jax.random.normal(self._next(), shape, dtype=jnp.bfloat16)
    def randint(self, lo, hi, shape):
        return jax.random.randint(self._next(), shape, lo, hi, dtype=jnp.int32)
    def uniform(self, shape, lo=0.0, hi=1.0):
        return jax.random.uniform(self._next(), shape, jnp.bfloat16, lo, hi)
    def permutation(self, n):
        return jax.random.permutation(self._next(), n)


kernel_name = 'concat_heads__mha_block_cached__mha_block_cached__near_ridge'

def setup_inputs():
    _rng = _Rng(jax.random.key(int.from_bytes(__import__("os").urandom(4), "little")))
    _w = (lambda a: (lambda t: t.astype(jnp.bfloat16) if jnp.issubdtype(t.dtype, jnp.floating) else t)(jnp.asarray(a)))
    def _A_setup():
        B, Sq, D = 16, 80, 512
        H, Sk, Dh = 32, 80, 128
        return {
            "x": _w((lambda *s: _rng.normal(s) * 0.8)(B, Sq, D)),
            "k_cache": _w((lambda *s: _rng.normal(s) * 0.8)(B, H, Sk, Dh)),
            "v_cache": _w((lambda *s: _rng.normal(s) * 0.05)(B, H, Sk, Dh)),
            "wq": _w((lambda *s: _rng.normal(s) * 0.8)(D, H * Dh) * (D ** -0.5)),
            "wo": _w((lambda *s: _rng.normal(s) * 0.05)(H * Dh, D) * ((H * Dh) ** -0.5)),
        }
    _A_in = _A_setup()

    def _B_setup():
        B, Sq, D = 16, 80, 512
        H, Sk, Dh = 32, 80, 128
        return {
            "x": _w((lambda *s: _rng.normal(s) * 0.8)(B, Sq, D)),
            "k_cache": _w((lambda *s: _rng.normal(s) * 0.8)(B, H, Sk, Dh)),
            "v_cache": _w((lambda *s: _rng.normal(s) * 0.05)(B, H, Sk, Dh)),
            "wq": _w((lambda *s: _rng.normal(s) * 0.8)(D, H * Dh) * (D ** -0.5)),
            "wo": _w((lambda *s: _rng.normal(s) * 0.05)(H * Dh, D) * ((H * Dh) ** -0.5)),
        }
    _B_in = _B_setup()

    return {
        "A_x": _A_in["x"],
        "A_k_cache": _A_in["k_cache"],
        "A_v_cache": _A_in["v_cache"],
        "A_wq": _A_in["wq"],
        "A_wo": _A_in["wo"],
        "B_x": _B_in["x"],
        "B_k_cache": _B_in["k_cache"],
        "B_v_cache": _B_in["v_cache"],
        "B_wq": _B_in["wq"],
        "B_wo": _B_in["wo"],
    }

def reference(A_x, A_k_cache, A_v_cache, A_wq, A_wo, B_x, B_k_cache, B_v_cache, B_wq, B_wo):
    def _A_ref(x, k_cache, v_cache, wq, wo):
        B, Sq, D = x.shape
        H, Dh = 32, 128
        q = (lambda x, *d: x.transpose(*d))((x @ wq).reshape(B, Sq, H, Dh), 0, 2, 1, 3)
        scores = jnp.einsum("bhqd,bhkd->bhqk", q, k_cache) * (Dh ** -0.5)
        p = _softmax(scores, axis=-1)
        o = jnp.einsum("bhqk,bhkd->bhqd", p, v_cache)
        return (lambda x, *d: x.transpose(*d))(o, 0, 2, 1, 3).reshape(B, Sq, H * Dh) @ wo

    def _B_ref(x, k_cache, v_cache, wq, wo):
        B, Sq, D = x.shape
        H, Dh = 32, 128
        q = (lambda x, *d: x.transpose(*d))((x @ wq).reshape(B, Sq, H, Dh), 0, 2, 1, 3)
        scores = jnp.einsum("bhqd,bhkd->bhqk", q, k_cache) * (Dh ** -0.5)
        p = _softmax(scores, axis=-1)
        o = jnp.einsum("bhqk,bhkd->bhqd", p, v_cache)
        return (lambda x, *d: x.transpose(*d))(o, 0, 2, 1, 3).reshape(B, Sq, H * Dh) @ wo

    a = _A_ref(A_x, A_k_cache, A_v_cache, A_wq, A_wo)
    b = _B_ref(B_x, B_k_cache, B_v_cache, B_wq, B_wo)
    return jnp.concatenate([a, b], axis=-1)
```

```python
import jax
import jax.numpy as jnp
import jax.experimental.pallas as pl
import jax.experimental.pallas.tpu as pltpu

B, SQ, D, H, SK, DH = 16, 80, 512, 32, 80, 128
M = B * SQ
HG = 4
W = HG * DH
NJ = H // HG
NSTEP = 2 * NJ
NQ = B // 4
NP = B // 2
NQLOOP, NMAIN = 3, 5
TQ0 = 2 + 3 * NQLOOP
EXP2_SCALE = DH ** -0.5 * 1.4426950408889634

f32, bf16, u32 = jnp.float32, jnp.bfloat16, jnp.uint32

USE = (((0, 1), (3, 1)), ((2, 1), (3, -1)), ((1, 1), (3, 1)), ((0, 1), (2, 1)),
       ((0, -1), (1, 1)), ((3, 1),), ((0, 1),))
NUSE = (4, 2, 2, 4)
ORDER = (1, 3, 0, 5, 2, 4, 6)


def _lhs_ops(a11, a12, a21, a22):
    return (a11 + a22, a21 + a22, a11, a22, a11 + a12, a21 - a11, a12 - a22)


def _rhs_ops(b11, b12, b21, b22):
    return (b11 + b22, b11, b12 - b22, b21 - b11, b22, b11 + b12, b21 + b22)


def _combine(state, m, val, emit):
    for c, sign in USE[m]:
        cur, cur_sign, count = state.get(c, (None, 1, 0))
        if cur is None:
            cur, cur_sign = val, sign
        elif cur_sign == sign:
            cur = cur + val
        elif cur_sign > 0:
            cur = cur - val
        else:
            cur, cur_sign = val - cur, 1
        if count + 1 == NUSE[c]:
            assert cur_sign == 1
            state.pop(c, None)
            emit(c, cur)
        else:
            state[c] = (cur, cur_sign, count + 1)


def _interleave(*streams):
    items = [((k + phase) / len(fs), n, k) for n, (phase, fs) in enumerate(streams) for k in range(len(fs))]
    for _, n, k in sorted(items):
        streams[n][1][k]()


def _nop():
    pass


def _pack(v):
    return pltpu.bitcast(v.astype(bf16), u32)


def _unpack(v):
    return pltpu.bitcast(v, bf16)


def _aligned(x, m):
    return x if isinstance(x, int) else pl.multiple_of(x, m)


def _tile(c):
    return slice(c * DH, (c + 1) * DH)


def _kernel(ax, ak, av, awq, awo, bx, bk, bv, bwq, bwo, out,
            xb, kb, vb, wqb, wob, xs, wqs, wos, q_s, o_s, acc, ob, sink, sinkf, in_sem, out_sem):
    xs_in, ks_in, vs_in, wqs_in, wos_in = (ax, bx), (ak, bk), (av, bv), (awq, bwq), (awo, bwo)

    def landing(kind, t, n):
        if kind == "x":
            return xb.at[t // NQ, pl.ds(t % NQ * 4 * SQ, n * 4 * SQ)]
        if kind == "wq":
            return wqb.at[:, pl.ds(_aligned(t * W, W), n * W)]
        if kind == "wo":
            return wob.at[pl.ds(_aligned(t * W, W), n * W)]
        return (kb if kind == "k" else vb).at[:, pl.ds(t * HG, n * HG)]

    def start(kind, t0, t1, s):
        if kind == "x":
            src = xs_in[t0 // NQ].at[pl.ds(t0 % NQ * 4 * SQ, (t1 - t0) * 4 * SQ)]
            pltpu.make_async_copy(src, landing("x", t0, t1 - t0), in_sem.at[s]).start()
            return
        for br in range(2):
            a, b = max(t0, br * NJ), min(t1, (br + 1) * NJ)
            if a < b:
                j, n = a - br * NJ, b - a
                if kind == "wq":
                    src = wqs_in[br].at[:, pl.ds(j * W, n * W)]
                elif kind == "wo":
                    src = wos_in[br].at[pl.ds(j * W, n * W)]
                else:
                    src = (ks_in if kind == "k" else vs_in)[br].at[:, pl.ds(j * HG, n * HG)]
                pltpu.make_async_copy(src, landing(kind, a, n), in_sem.at[s]).start()

    def wait(kind, t, n, s):
        dst = landing(kind, t, n)
        pltpu.make_async_copy(dst, dst, in_sem.at[s]).wait()

    def wprep(is_q, t, slot):
        def chunk(r0):
            if is_q:
                raw = [[wqb[r * DH + r0:r * DH + r0 + 16, pl.ds(_aligned(t * W + c * DH, DH), DH)]
                        for c in range(4)] for r in range(4)]
            else:
                raw = [[wob[pl.ds(_aligned(t * W + r * DH + r0, 16), 16), _tile(c)]
                        for c in range(4)] for r in range(4)]
            raw = [[v.astype(f32) for v in row] for row in raw]
            for r in range(2):
                w0 = (r * DH + r0) // 2
                for c in range(2):
                    for m, v in enumerate(_rhs_ops(raw[r][c], raw[r][2 + c], raw[2 + r][c], raw[2 + r][2 + c])):
                        (wqs if is_q else wos)[slot, m, c, w0:w0 + 8, :] = _pack(v)
        return [lambda r0=r0: chunk(r0) for r0 in range(0, DH, 16)]

    def xprep(br, i):
        def chunk(p, r0):
            raw = [[xb[br, (2 * p + r) * SQ + r0:(2 * p + r) * SQ + r0 + 16, _tile(c)].astype(f32)
                    for c in range(4)] for r in range(2)]
            for c in range(2):
                for m, v in enumerate(_lhs_ops(raw[0][c], raw[0][2 + c], raw[1][c], raw[1][2 + c])):
                    xs[p, m, c, r0 // 2:r0 // 2 + 8, :] = _pack(v)
        return [lambda p=p, r0=r0: chunk(p, r0) for p in (2 * i, 2 * i + 1) for r0 in range(0, SQ, 16)]

    def early(fs, i):
        return fs[(0, 3, 6, 8)[i]:(3, 6, 8, 8)[i]]

    def wide(ref, *idx):
        return jnp.concatenate([_unpack(ref[idx + (0,)]), _unpack(ref[idx + (1,)])], axis=1)

    def products(i, one):
        return [lambda p=p, c=c, m=m: one(p, c, m) for p in (2 * i, 2 * i + 1) for c in range(2) for m in ORDER]

    def project_q(t, i, slot):
        state = {}

        def one(p, c, m):
            def emit(u, v):
                q_s[t, 2 * p + u // 2, u % 2 * 2 + c] = _pack(v)
            _combine(state, m, jnp.dot(wide(xs, p, m), _unpack(wqs[slot, m, c]), preferred_element_type=f32), emit)
        return products(i, one)

    def heads(p, c):
        return ((2 * p, c), (2 * p, 2 + c), (2 * p + 1, c), (2 * p + 1, 2 + c))

    def scores(t, i, probs):
        def one(p, c):
            for b, h in heads(p, c):
                s = jax.lax.dot_general(_unpack(q_s[t, b, h]), kb[b, t * HG + h], (((1,), (1,)), ((), ())),
                                        preferred_element_type=f32)
                e = jnp.exp2((s - jnp.max(s, axis=1, keepdims=True)) * EXP2_SCALE)
                total = jnp.sum(e, axis=1, keepdims=True)
                probs[b, h] = (e * pl.reciprocal(total, approx=True)).astype(bf16)
        return [lambda p=p, c=c: one(p, c) for p in (2 * i, 2 * i + 1) for c in range(2)]

    def attend(t, i, probs, slot):
        def one(p, c):
            o = [jnp.dot(probs.pop((b, h)), vb[b, t * HG + h], preferred_element_type=f32) for b, h in heads(p, c)]
            for m, v in enumerate(_lhs_ops(*o)):
                o_s[slot, p % 2, m, c] = _pack(v)
        return [lambda p=p, c=c: one(p, c) for p in (2 * i, 2 * i + 1) for c in range(2)]

    def project_out(t, i, slot, wslot, keep=True, emit=False, may_restart=False):
        state = {}

        def one(p, c, m):
            def write(u, v):
                r0 = (2 * p + u // 2) * SQ
                ob[t // NJ, r0:r0 + SQ, _tile(u % 2 * 2 + c)] = v.astype(bf16)
            old = acc[p, m, c]
            if may_restart:
                old = jnp.where(t % NJ == 0, 0.0, old)
            val = old + jnp.dot(wide(o_s, slot, p % 2, m), _unpack(wos[wslot, m, c]), preferred_element_type=f32)
            if keep:
                acc[p, m, c] = val
            if emit:
                _combine(state, m, val, write)
        return products(i, one)

    pending = []

    def copy_out(src, dst):
        c = pltpu.make_async_copy(src, dst, out_sem.at[len(pending)])
        c.start()
        pending.append(c)

    def put(br, p0, p1):
        rows = pl.ds(p0 * 2 * SQ, (p1 - p0) * 2 * SQ)
        copy_out(ob.at[br, rows], out.at[rows, pl.ds(br * D, D)])

    start("wq", 0, 1, 0)
    start("x", 0, 1, 1)
    start("x", 1, 3, 2)
    start("x", 3, 4, 3)
    start("wq", 1, 2, 4)
    start("wq", 2, 3, 5)
    start("wq", 3, 6, 7)
    start("x", NQ, 2 * NQ, 6)
    start("wq", 6, 9, 8)
    start("wq", 9, 12, 9)
    start("wq", 12, NSTEP, 10)
    for n in range(NMAIN):
        t1 = 3 * n + 3 if n < NMAIN - 1 else NSTEP
        for k, kind in enumerate(("wo", "k", "v")):
            start(kind, 3 * n, t1, 11 + 3 * n + k)
    acc[...] = jnp.zeros(acc.shape, f32)

    wait("wq", 0, 1, 0)
    wait("x", 0, 1, 1)
    _interleave((0, wprep(True, 0, 1)), (0, xprep(0, 0)))
    for g in range(2 * NQ):
        t, i = divmod(g, NQ)
        extra = []
        if g == 1:
            wait("x", 1, 2, 2)
            _interleave((0, xprep(0, 1)))
            extra = xprep(0, 2)
        if g == 3:
            wait("x", 3, 1, 3)
            wait("wq", 1, 1, 4)
            _interleave((0, xprep(0, 3)))
            extra = wprep(True, 1, 2) + [_nop] * 3
        if g == 7:
            wait("wq", 2, 1, 5)
            extra = wprep(True, 2, 0)
        _interleave((0.5, project_q(t, i, (t + 1) % 3)), (0, extra))

    def q_body(n, _):
        @pl.when(n == 1)
        def _():
            wait("x", NQ, NQ, 6)
        wait("wq", 3 + 3 * n, 3, 7 + n)
        for s in range(3):
            t = 2 + 3 * n + s
            w = wprep(True, t + 1, (s + 1) % 3)
            for i in range(NQ):
                if s == 0:
                    extra = (xprep(n // 2, NQ - 1), w[:4], w[4:], [])[i]
                elif s == 1:
                    extra = early(w, i)
                else:
                    extra = w if i == 0 else xprep(jnp.minimum(n, 1), i - 1) + [_nop] * (4 if i == 3 else 0)
                _interleave((0.5, project_q(t, i, s)), (0, extra))

    jax.lax.fori_loop(0, NQLOOP, q_body, None)
    wait("wq", 12, NSTEP - 12, 10)

    def main_body(n, _):
        def arrive(count):
            for k, kind in enumerate(("wo", "k", "v")):
                wait(kind, 3 * n, count, 11 + 3 * n + k)
        jax.lax.cond(n < NMAIN - 1, lambda: arrive(3), lambda: arrive(4))
        tq = TQ0 + n
        at = lambda g: (3 * n + g // NQ, g % NQ)
        probs = [{} for _ in range(3 * NQ)]
        _interleave((0, scores(*at(0), probs[0]) + scores(*at(1), probs[1])))
        _interleave((0, project_q(tq, 0, 0) + project_q(tq, 1, 0)), (0.5, wprep(False, 3 * n, 0)))
        _interleave((0.5, project_q(tq, 2, 0)), (0.5, attend(*at(0), probs[0], 0)))
        _interleave((0.5, project_q(tq, 3, 0)))
        wq_next = wprep(True, jnp.minimum(tq + 1, NSTEP - 1), 0)
        for g in range(3 * NQ):
            (t, i), s = at(g), g // NQ
            streams = [(0.1, project_out(t, i, g % 2, s, emit=s == 1, may_restart=s == 2))]
            if s < 2:
                streams.append((0.5, early(wprep(False, t + 1, s + 1), i)))
            if g + 1 < 3 * NQ:
                streams.append((0.4, attend(*at(g + 1), probs[g + 1], (g + 1) % 2)))
            if g + 2 < 3 * NQ:
                streams.append((0.9, scores(*at(g + 2), probs[g + 2])))
            if s == 2:
                streams.append((0.2, wq_next[2 * i:2 * i + 2]))
            _interleave(*streams)

    jax.lax.fori_loop(0, NMAIN, main_body, None)

    t = NSTEP - 1
    put(0, 0, NP)
    probs = [{} for _ in range(NQ)]
    _interleave((0, scores(t, 0, probs[0]) + scores(t, 1, probs[1]) + scores(t, 2, probs[2])
                 + attend(t, 0, probs[0], 0) + attend(t, 1, probs[1], 1)), (0, wprep(False, t, 0)))
    sent = 0
    for i in range(NQ):
        o = project_out(t, i, i % 3, 0, keep=False, emit=True)
        s = scores(t, 3, probs[3]) if i == 0 else []
        a = attend(t, i + 2, probs[i + 2], (i + 2) % 3) if i + 2 < NQ else []
        for h in range(2):
            _interleave((0.1, o[h * 14:h * 14 + 14]), (0, s[2 * h:2 * h + 2]), (0.5, a[2 * h:2 * h + 2]))
            if 2 * i + h + 1 in (4, 7, NP):
                put(1, sent, 2 * i + h + 1)
                sent = 2 * i + h + 1

    for n, src in enumerate((wqs.at[0, 0, 0, :8], wos.at[0, 0, 0, :8], xs.at[0, 0, 0, :8],
                             q_s.at[0, 0, 0, :8], o_s.at[0, 0, 0, 0, :8])):
        copy_out(src, sink.at[n])
    copy_out(acc.at[0, 0, 0, :8], sinkf)
    for c in pending:
        c.wait()


@jax.jit
def pallas_concat_heads__mha_block_cached__mha_block_cached__near_ridge_kernel(
    A_x: jax.Array,
    A_k_cache: jax.Array,
    A_v_cache: jax.Array,
    A_wq: jax.Array,
    A_wo: jax.Array,
    B_x: jax.Array,
    B_k_cache: jax.Array,
    B_v_cache: jax.Array,
    B_wq: jax.Array,
    B_wo: jax.Array,
):
    out = pl.pallas_call(
        _kernel,
        in_specs=[pl.BlockSpec(memory_space=pl.ANY)] * 10,
        out_specs=pl.BlockSpec(memory_space=pl.ANY),
        out_shape=jax.ShapeDtypeStruct((M, 2 * D), bf16),
        scratch_shapes=[
            pltpu.VMEM((2, M, D), bf16),
            pltpu.VMEM((B, 2 * H, SK, DH), bf16),
            pltpu.VMEM((B, 2 * H, SK, DH), bf16),
            pltpu.VMEM((D, 2 * H * DH), bf16),
            pltpu.VMEM((2 * H * DH, D), bf16),
            pltpu.VMEM((NP, 7, 2, SQ // 2, DH), u32),
            pltpu.VMEM((3, 7, 2, DH, DH), u32),
            pltpu.VMEM((3, 7, 2, DH, DH), u32),
            pltpu.VMEM((NSTEP, B, HG, SQ // 2, DH), u32),
            pltpu.VMEM((3, 2, 7, 2, SQ // 2, DH), u32),
            pltpu.VMEM((NP, 7, 2, SQ, DH), f32),
            pltpu.VMEM((2, M, D), bf16),
            pltpu.VMEM((5, 8, DH), u32),
            pltpu.VMEM((8, DH), f32),
            pltpu.SemaphoreType.DMA((11 + 3 * NMAIN,)),
            pltpu.SemaphoreType.DMA((10,)),
        ],
        compiler_params=pltpu.CompilerParams(vmem_limit_bytes=124 * 1024 * 1024),
    )(A_x.reshape(M, D), A_k_cache, A_v_cache, A_wq, A_wo,
      B_x.reshape(M, D), B_k_cache, B_v_cache, B_wq, B_wo)
    return out.reshape(B, SQ, 2 * D)
```

```python
import jax
import jax.numpy as jnp
import jax.experimental.pallas as pl
import jax.experimental.pallas.tpu as pltpu

B, SQ, D, H, SK, DH = 16, 80, 512, 32, 80, 128
M = B * SQ
HG = 4
W = HG * DH
NJ = H // HG
NSTEP = 2 * NJ
NQ = B // 4
NP = B // 2
NQLOOP, NMAIN = 3, 5
TQ0 = 2 + 3 * NQLOOP
EXP2_SCALE = DH ** -0.5 * 1.4426950408889634

f32, bf16, u32 = jnp.float32, jnp.bfloat16, jnp.uint32

USE = (((0, 1), (3, 1)), ((2, 1), (3, -1)), ((1, 1), (3, 1)), ((0, 1), (2, 1)),
       ((0, -1), (1, 1)), ((3, 1),), ((0, 1),))
NUSE = (4, 2, 2, 4)
ORDER = (1, 3, 0, 5, 2, 4, 6)


def _lhs_ops(a11, a12, a21, a22):
    return (a11 + a22, a21 + a22, a11, a22, a11 + a12, a21 - a11, a12 - a22)


def _rhs_ops(b11, b12, b21, b22):
    return (b11 + b22, b11, b12 - b22, b21 - b11, b22, b11 + b12, b21 + b22)


def _combine(state, m, val, emit):
    for c, sign in USE[m]:
        cur, cur_sign, count = state.get(c, (None, 1, 0))
        if cur is None:
            cur, cur_sign = val, sign
        elif cur_sign == sign:
            cur = cur + val
        elif cur_sign > 0:
            cur = cur - val
        else:
            cur, cur_sign = val - cur, 1
        if count + 1 == NUSE[c]:
            assert cur_sign == 1
            state.pop(c, None)
            emit(c, cur)
        else:
            state[c] = (cur, cur_sign, count + 1)


def _interleave(*streams):
    items = [((k + phase) / len(fs), n, k) for n, (phase, fs) in enumerate(streams) for k in range(len(fs))]
    for _, n, k in sorted(items):
        streams[n][1][k]()


def _nop():
    pass


def _pack(v):
    return pltpu.bitcast(v.astype(bf16), u32)


def _unpack(v):
    return pltpu.bitcast(v, bf16)


def _aligned(x, m):
    return x if isinstance(x, int) else pl.multiple_of(x, m)


def _tile(c):
    return slice(c * DH, (c + 1) * DH)


def _kernel(ax, ak, av, awq, awo, bx, bk, bv, bwq, bwo, out,
            xb, kb, vb, wqb, wob, xs, wqs, wos, q_s, o_s, acc, ob, sink, sinkf, in_sem, out_sem):
    xs_in, ks_in, vs_in, wqs_in, wos_in = (ax, bx), (ak, bk), (av, bv), (awq, bwq), (awo, bwo)

    def landing(kind, t, n):
        if kind == "x":
            return xb.at[t // NP, pl.ds(t % NP * 2 * SQ, n * 2 * SQ)]
        if kind == "wq":
            return wqb.at[:, pl.ds(_aligned(t * W, W), n * W)]
        if kind == "wo":
            return wob.at[pl.ds(_aligned(t * W, W), n * W)]
        return (kb if kind == "k" else vb).at[:, pl.ds(t * HG, n * HG)]

    def start(kind, t0, t1, s):
        if kind == "x":
            src = xs_in[t0 // NP].at[pl.ds(t0 % NP * 2 * SQ, (t1 - t0) * 2 * SQ)]
            pltpu.make_async_copy(src, landing("x", t0, t1 - t0), in_sem.at[s]).start()
            return
        for br in range(2):
            a, b = max(t0, br * NJ), min(t1, (br + 1) * NJ)
            if a < b:
                j, n = a - br * NJ, b - a
                if kind == "wq":
                    src = wqs_in[br].at[:, pl.ds(j * W, n * W)]
                elif kind == "wo":
                    src = wos_in[br].at[pl.ds(j * W, n * W)]
                else:
                    src = (ks_in if kind == "k" else vs_in)[br].at[:, pl.ds(j * HG, n * HG)]
                pltpu.make_async_copy(src, landing(kind, a, n), in_sem.at[s]).start()

    def wait(kind, t, n, s):
        dst = landing(kind, t, n)
        pltpu.make_async_copy(dst, dst, in_sem.at[s]).wait()

    def wprep(is_q, t, slot):
        def chunk(r0):
            if is_q:
                raw = [[wqb[r * DH + r0:r * DH + r0 + 16, pl.ds(_aligned(t * W + c * DH, DH), DH)]
                        for c in range(4)] for r in range(4)]
            else:
                raw = [[wob[pl.ds(_aligned(t * W + r * DH + r0, 16), 16), _tile(c)]
                        for c in range(4)] for r in range(4)]
            raw = [[v.astype(f32) for v in row] for row in raw]
            for r in range(2):
                w0 = (r * DH + r0) // 2
                for c in range(2):
                    for m, v in enumerate(_rhs_ops(raw[r][c], raw[r][2 + c], raw[2 + r][c], raw[2 + r][2 + c])):
                        (wqs if is_q else wos)[slot, m, c, w0:w0 + 8, :] = _pack(v)
        return [lambda r0=r0: chunk(r0) for r0 in range(0, DH, 16)]

    def xprep(br, i):
        def chunk(p, r0):
            raw = [[xb[br, (2 * p + r) * SQ + r0:(2 * p + r) * SQ + r0 + 16, _tile(c)].astype(f32)
                    for c in range(4)] for r in range(2)]
            for c in range(2):
                for m, v in enumerate(_lhs_ops(raw[0][c], raw[0][2 + c], raw[1][c], raw[1][2 + c])):
                    xs[p, m, c, r0 // 2:r0 // 2 + 8, :] = _pack(v)
        return [lambda p=p, r0=r0: chunk(p, r0) for p in (2 * i, 2 * i + 1) for r0 in range(0, SQ, 16)]

    def early(fs, i):
        return fs[(0, 3, 6, 8)[i]:(3, 6, 8, 8)[i]]

    def wide(ref, *idx):
        return jnp.concatenate([_unpack(ref[idx + (0,)]), _unpack(ref[idx + (1,)])], axis=1)

    def products(i, one):
        return [lambda p=p, c=c, m=m: one(p, c, m) for p in (2 * i, 2 * i + 1) for c in range(2) for m in ORDER]

    def project_q(t, i, slot):
        state = {}

        def one(p, c, m):
            def emit(u, v):
                q_s[t, 2 * p + u // 2, u % 2 * 2 + c] = _pack(v)
            _combine(state, m, jnp.dot(wide(xs, p, m), _unpack(wqs[slot, m, c]), preferred_element_type=f32), emit)
        return products(i, one)

    def heads(p, c):
        return ((2 * p, c), (2 * p, 2 + c), (2 * p + 1, c), (2 * p + 1, 2 + c))

    def scores(t, i, probs):
        def one(p, c):
            for b, h in heads(p, c):
                s = jax.lax.dot_general(_unpack(q_s[t, b, h]), kb[b, t * HG + h], (((1,), (1,)), ((), ())),
                                        preferred_element_type=f32)
                e = jnp.exp2((s - jnp.max(s, axis=1, keepdims=True)) * EXP2_SCALE)
                total = jnp.sum(e, axis=1, keepdims=True)
                probs[b, h] = (e * pl.reciprocal(total, approx=True)).astype(bf16)
        return [lambda p=p, c=c: one(p, c) for p in (2 * i, 2 * i + 1) for c in range(2)]

    def attend(t, i, probs, slot):
        def one(p, c):
            o = [jnp.dot(probs.pop((b, h)), vb[b, t * HG + h], preferred_element_type=f32) for b, h in heads(p, c)]
            for m, v in enumerate(_lhs_ops(*o)):
                o_s[slot, p % 2, m, c] = _pack(v)
        return [lambda p=p, c=c: one(p, c) for p in (2 * i, 2 * i + 1) for c in range(2)]

    def project_out(t, i, slot, wslot, keep=True, emit=False, may_restart=False):
        state = {}

        def one(p, c, m):
            def write(u, v):
                r0 = (2 * p + u // 2) * SQ
                ob[t // NJ, r0:r0 + SQ, _tile(u % 2 * 2 + c)] = v.astype(bf16)
            old = acc[p, m, c]
            if may_restart:
                old = jnp.where(t % NJ == 0, 0.0, old)
            val = old + jnp.dot(wide(o_s, slot, p % 2, m), _unpack(wos[wslot, m, c]), preferred_element_type=f32)
            if keep:
                acc[p, m, c] = val
            if emit:
                _combine(state, m, val, write)
        return products(i, one)

    pending = []

    def copy_out(src, dst):
        c = pltpu.make_async_copy(src, dst, out_sem.at[len(pending)])
        c.start()
        pending.append(c)

    def put(br, p0, p1):
        rows = pl.ds(p0 * 2 * SQ, (p1 - p0) * 2 * SQ)
        copy_out(ob.at[br, rows], out.at[rows, pl.ds(br * D, D)])

    start("wq", 0, 1, 0)
    x_parts = {0: (1, 1), 1: (2, 2), 3: (4, 3), 7: (1, 4)}
    for p, (count, s) in x_parts.items():
        start("x", p, p + count, s)
    start("wq", 1, 3, 5)
    start("wq", 3, 6, 7)
    start("x", NP, 2 * NP, 6)
    start("wq", 6, 9, 8)
    start("wq", 9, 12, 9)
    start("wq", 12, NSTEP, 10)
    for n in range(NMAIN):
        for k, kind in enumerate(("wo", "k", "v")):
            start(kind, 3 * n, 3 * n + 3, 11 + 3 * n + k)
    acc[...] = jnp.zeros(acc.shape, f32)

    wait("wq", 0, 1, 0)
    x_ops = [f for i in range(NQ) for f in xprep(0, i)]
    step0 = [f for i in range(NQ) for f in project_q(0, i, 1)]
    for p in range(NP):
        if p in x_parts:
            wait("x", p, *x_parts[p])
            if p == NP - 1:
                wait("wq", 1, 2, 5)
            _interleave((0, wprep(True, 0, 1) if p == 0 else []), (0, x_ops[5 * p:5 * p + 5]))
        extra = [] if p + 1 in x_parts else x_ops[5 * p + 5:5 * p + 10]
        if p == NP - 1:
            extra = wprep(True, 1, 2) + [_nop] * 2
        _interleave((0.5, step0[14 * p:14 * p + 14]), (0, extra))
    for i in range(NQ):
        _interleave((0.5, project_q(1, i, 2)), (0, early(wprep(True, 2, 0), i)))

    def q_body(n, _):
        wait("wq", 3 + 3 * n, 3, 7 + n)
        zero = n // 8
        for s in range(3):
            t = 2 + 3 * n + s
            w = wprep(True, t + 1, (s + 1) % 3)
            for i in range(NQ):
                if s == 0:
                    extra = (xprep(n // 2, NQ - 1), w[:4], w[4:], [])[i]
                elif s == 1:
                    extra = early(w, i)
                else:
                    extra = w if i == 0 else xprep(jnp.minimum(n, 1), i - 1) + [_nop] * (4 if i == 3 else 0)
                _interleave((0.5, project_q(t, i, s + zero)), (0, extra))

    wait("x", NP, NP, 6)
    jax.lax.fori_loop(0, NQLOOP, q_body, None)
    wait("wq", 12, NSTEP - 12, 10)
    for k, kind in enumerate(("wo", "k", "v")):
        start(kind, NSTEP - 1, NSTEP, 11 + 3 * NMAIN + k)

    def main_body(n, _):
        for k, kind in enumerate(("wo", "k", "v")):
            wait(kind, 3 * n, 3, 11 + 3 * n + k)
        tq = TQ0 + n
        at = lambda g: (3 * n + g // NQ, g % NQ)
        probs = [{} for _ in range(3 * NQ)]
        _interleave((0, scores(*at(0), probs[0]) + scores(*at(1), probs[1])))
        _interleave((0, project_q(tq, 0, 0) + project_q(tq, 1, 0)), (0.5, wprep(False, 3 * n, 0)))
        _interleave((0.5, project_q(tq, 2, 0)), (0.5, attend(*at(0), probs[0], 0)))
        _interleave((0.5, project_q(tq, 3, 0)))
        wq_next = wprep(True, jnp.minimum(tq + 1, NSTEP - 1), 0)
        for g in range(3 * NQ):
            (t, i), s = at(g), g // NQ
            streams = [(0.1, project_out(t, i, g % 2, s, emit=s == 1, may_restart=s == 2))]
            if s < 2:
                streams.append((0.5, early(wprep(False, t + 1, s + 1), i)))
            if g + 1 < 3 * NQ:
                streams.append((0.4, attend(*at(g + 1), probs[g + 1], (g + 1) % 2)))
            if g + 2 < 3 * NQ:
                streams.append((0.9, scores(*at(g + 2), probs[g + 2])))
            if s == 2:
                streams.append((0.2, wq_next[2 * i:2 * i + 2]))
            _interleave(*streams)

    jax.lax.fori_loop(0, NMAIN, main_body, None)

    t = NSTEP - 1
    put(0, 0, NP)
    for k, kind in enumerate(("wo", "k", "v")):
        wait(kind, t, 1, 11 + 3 * NMAIN + k)
    probs = [{} for _ in range(NQ)]
    _interleave((0, scores(t, 0, probs[0]) + scores(t, 1, probs[1]) + attend(t, 0, probs[0], 0)
                 + scores(t, 2, probs[2])), (0, wprep(False, t, 0)))
    sent = 0
    for i in range(NQ):
        o = project_out(t, i, i % 3, 0, keep=False, emit=True)
        s = scores(t, 3, probs[3]) if i == 0 else []
        a = attend(t, i + 1, probs[i + 1], (i + 1) % 3) if i + 1 < NQ else []
        for h in range(2):
            _interleave((0.1, o[h * 14:h * 14 + 14]), (0, s[2 * h:2 * h + 2]), (0.5, a[2 * h:2 * h + 2]))
            if 2 * i + h + 1 in (2, 4, 6, 7, NP):
                put(1, sent, 2 * i + h + 1)
                sent = 2 * i + h + 1

    for n, src in enumerate((wqs.at[0, 0, 0, :8], wos.at[0, 0, 0, :8], xs.at[0, 0, 0, :8],
                             q_s.at[0, 0, 0, :8], o_s.at[0, 0, 0, 0, :8])):
        copy_out(src, sink.at[n])
    copy_out(acc.at[0, 0, 0, :8], sinkf)
    for c in pending:
        c.wait()


@jax.jit
def pallas_concat_heads__mha_block_cached__mha_block_cached__near_ridge_kernel(
    A_x: jax.Array,
    A_k_cache: jax.Array,
    A_v_cache: jax.Array,
    A_wq: jax.Array,
    A_wo: jax.Array,
    B_x: jax.Array,
    B_k_cache: jax.Array,
    B_v_cache: jax.Array,
    B_wq: jax.Array,
    B_wo: jax.Array,
):
    out = pl.pallas_call(
        _kernel,
        in_specs=[pl.BlockSpec(memory_space=pl.ANY)] * 10,
        out_specs=pl.BlockSpec(memory_space=pl.ANY),
        out_shape=jax.ShapeDtypeStruct((M, 2 * D), bf16),
        scratch_shapes=[
            pltpu.VMEM((2, M, D), bf16),
            pltpu.VMEM((B, 2 * H, SK, DH), bf16),
            pltpu.VMEM((B, 2 * H, SK, DH), bf16),
            pltpu.VMEM((D, 2 * H * DH), bf16),
            pltpu.VMEM((2 * H * DH, D), bf16),
            pltpu.VMEM((NP, 7, 2, SQ // 2, DH), u32),
            pltpu.VMEM((3, 7, 2, DH, DH), u32),
            pltpu.VMEM((3, 7, 2, DH, DH), u32),
            pltpu.VMEM((NSTEP, B, HG, SQ // 2, DH), u32),
            pltpu.VMEM((3, 2, 7, 2, SQ // 2, DH), u32),
            pltpu.VMEM((NP, 7, 2, SQ, DH), f32),
            pltpu.VMEM((2, M, D), bf16),
            pltpu.VMEM((5, 8, DH), u32),
            pltpu.VMEM((8, DH), f32),
            pltpu.SemaphoreType.DMA((14 + 3 * NMAIN,)),
            pltpu.SemaphoreType.DMA((12,)),
        ],
        compiler_params=pltpu.CompilerParams(vmem_limit_bytes=124 * 1024 * 1024),
    )(A_x.reshape(M, D), A_k_cache, A_v_cache, A_wq, A_wo,
      B_x.reshape(M, D), B_k_cache, B_v_cache, B_wq, B_wo)
    return out.reshape(B, SQ, 2 * D)
```
